```python
import os as _os
_os.environ.setdefault("JAX_PLATFORMS", "cpu")
import jax
import jax.numpy as jnp

def _softmax(x, axis=-1):
    return jax.nn.softmax(x, axis=axis)
def _gelu(x):
    return jax.nn.gelu(x, approximate=True)
def _silu(x):
    return jax.nn.silu(x)
def _sigmoid(x):
    return jax.nn.sigmoid(x)
def _layernorm(x, axis=-1, eps=1e-5):
    m = jnp.mean(x, axis=axis, keepdims=True)
    v = jnp.var(x, axis=axis, keepdims=True)
    return (x - m) / jnp.sqrt(v + eps)
def _scatter_add(tgt, idx, src, axis=0):
    return tgt.at[idx].add(src)
def _segment_sum(src, seg, n):
    return jax.ops.segment_sum(src, seg, n)
class _Rng:
    def __init__(self, key):
        self._k = key
    def _next(self):
        self._k, sub = jax.random.split(self._k)
        return sub
    def normal(self, shape):
        return jax.random.normal(self._next(), shape, dtype=jnp.bfloat16)
    def randint(self, lo, hi, shape):
        return jax.random.randint(self._next(), shape, lo, hi, dtype=jnp.int32)
    def uniform(self, shape, lo=0.0, hi=1.0):
        return jax.random.uniform(self._next(), shape, jnp.bfloat16, lo, hi)
    def permutation(self, n):
        return jax.random.permutation(self._next(), n)


kernel_name = 'standalone__seq2seq_rnn_t_joint__speech'

def setup_inputs():
    _rng = _Rng(jax.random.key(int.from_bytes(__import__("os").urandom(4), "little")))
    _w = (lambda a: (lambda t: t.astype(jnp.bfloat16) if jnp.issubdtype(t.dtype, jnp.floating) else t)(jnp.asarray(a)))
    B, T, D, K = 2, 1000, 512, 31
    U = 8
    sc = (1.0 / (K * D)) ** 0.5
    sd = (1.0 / D) ** 0.5
    return {
        "x": _w((lambda *s: _rng.normal(s) * 0.4)(B, T, D) * 0.5),
        "w1": _w((lambda *s: _rng.normal(s) * 1.6)(K, D, D) * sc),
        "w2": _w((lambda *s: _rng.normal(s) * 1.6)(K, D, D) * sc),
        "g": _w((lambda *s: _rng.normal(s) * 1.6)(B, U, D) * 0.5),
        "w_f": _w((lambda *s: _rng.normal(s) * 1.6)(D, D) * sd),
        "w_g": _w((lambda *s: _rng.normal(s) * 1.6)(D, D) * sd),
        "w_o": _w((lambda *s: _rng.normal(s) * 1.6)(D, D) * sd),
    }

def reference(x, w1, w2, g, w_f, w_g, w_o):
    B, T, D = x.shape
    K = w1.shape[0]
    pad = K // 2
    xp = jnp.pad(x, ((0,0),(pad,pad),(0,0)))
    h = jnp.zeros_like(x)
    for i in range(K):
        h = h + jnp.einsum("btc,cd->btd", xp[:, i:i+T, :], w1[i])
    h = _gelu(h)[:, ::2, :]
    T1 = h.shape[1]
    hp = jnp.pad(h, ((0,0),(pad,pad),(0,0)))
    f = jnp.zeros_like(h)
    for i in range(K):
        f = f + jnp.einsum("btc,cd->btd", hp[:, i:i+T1, :], w2[i])
    f = _gelu(f)[:, ::2, :]
    fe = jnp.einsum("btd,de->bte", f, w_f)
    ge = jnp.einsum("bud,de->bue", g, w_g)
    j = jnp.tanh(fe[:, :, None, :] + ge[:, None, :, :])
    return jnp.einsum("btud,dv->btuv", j, w_o)
```

```python
import functools

import jax
import jax.numpy as jnp
import jax.experimental.pallas as pl
import jax.experimental.pallas.tpu as pltpu

_L1 = 4
_L2 = 3
_NCH = 4
_BAR = 2
_S = 32


def _in_tree(u, lv, emit, base=0):
  if lv == 0:
    emit(base, u[0]())
    return
  h = 1 << (lv - 1)
  n = 2 * h - 1
  k = 3 ** (lv - 1)
  keep = lambda v: (lambda: v)
  _in_tree([keep(u[q]() - u[q + h]()) for q in range(n)], lv - 1, emit, base)
  _in_tree([u[q + h] for q in range(n)], lv - 1, emit, base + k)
  _in_tree([keep(u[q + 2 * h]() - u[q + h]()) for q in range(n)], lv - 1, emit,
           base + 2 * k)


def _out_tree(m, lv):
  if lv == 0:
    return [m[0]()]
  n = 3 ** (lv - 1)
  a = _out_tree(m[:n], lv - 1)
  b = _out_tree(m[n:2 * n], lv - 1)
  ab = [p + q for p, q in zip(a, b)]
  c = _out_tree(m[2 * n:], lv - 1)
  return ab + [p + q for p, q in zip(c, b)]


def _w_sets(lv):
  def rec(w, l):
    if l == 0:
      return list(w)
    h = 1 << (l - 1)
    we, wo = w[:h], w[h:]
    return rec(we, l - 1) + rec([a | b for a, b in zip(we, wo)], l - 1) + rec(wo, l - 1)
  return rec([frozenset([i]) for i in range(1 << lv)], lv)


def _w_tree(get, lv, emit):
  def rec(w, l, base, raw):
    if l == 0:
      if not raw:
        emit(base, w[0]())
      return
    h = 1 << (l - 1)
    n = 3 ** (l - 1)
    we, wo = w[:h], w[h:]
    rec(we, l - 1, base, raw)
    ws = []
    for a, b in zip(we, wo):
      (a0, a1), (b0, b1) = a(), b()
      ws.append(functools.partial(lambda v: v, (a0 + b0, a1 + b1)))
    rec(ws, l - 1, base + n, False)
    rec(wo, l - 1, base + 2 * n, raw)
  rec([functools.lru_cache(None)(functools.partial(get, i)) for i in range(1 << lv)],
      lv, 0, True)


def _gelu(x):
  c = 0.7978845608028654
  return 0.5 * x * (1.0 + jnp.tanh(c * (x + 0.044715 * (x * x * x))))


def _lo(v):
  return pltpu.bitcast(v << 16, jnp.float32)


def _hi(v):
  return pltpu.bitcast(v & jnp.uint32(0xFFFF0000), jnp.float32)


@jax.jit
def pallas_standalone__seq2seq_rnn_t_joint__speech_kernel(
    x: jax.Array,
    w1: jax.Array,
    w2: jax.Array,
    g: jax.Array,
    w_f: jax.Array,
    w_g: jax.Array,
    w_o: jax.Array,
):
  B, T, D = x.shape
  K = w1.shape[0]
  U = g.shape[1]
  assert (B, T, D, K, U) == (2, 1000, 512, 31, 8)
  T1, T2 = T // 2, T // 4
  bf16, f32, u32 = jnp.bfloat16, jnp.float32, jnp.uint32
  M = B * _S
  NCH = _NCH
  XROWS = 528

  def make_sum_index(lv):
    sets = _w_sets(lv)
    idx, k = {}, 0
    for c, s in enumerate(sets):
      if len(s) > 1:
        idx[c] = k
        k += 1
    return sets, idx, k

  sets1, sidx1, ns1 = make_sum_index(_L1)
  sets2, sidx2, ns2 = make_sum_index(_L2)
  A1, A2 = 16 >> _L1, 16 >> _L2
  NSUM = max(ns1 * A1, ns2 * A2)

  def kernel(x_hbm, w1_hbm, w2_hbm, g_hbm, wf_hbm, wg_hbm, wo_hbm, o_hbm,
             xb, w1b, w2b, ws, xl1, xl2, macc, hb, fb, fe, gb, wfb, wgb, wob, ob,
             sem_x, sem_w, sem_s, sem_o, sm):
    sm[0] = K + 1
    sm[1] = 0
    zi = jax.lax.fori_loop(0, sm[1] + 1, lambda i, v: v + i, sm[0])
    zr = pl.multiple_of(jax.lax.fori_loop(0, sm[1] + 1, lambda i, v: v + i, sm[1]), 8)
    zm = zi + (3 ** _L1 - K - 1)
    zh = zi - (K + 1 - 16)
    def x_copy(b, c):
      return pltpu.make_async_copy(
          x_hbm.at[b, :, pl.ds(c * 128, 128)], xb.bitcast(bf16).at[b, c, pl.ds(16, T), :],
          sem_x.at[b * NCH + c])

    def w_copy(layer, n, c):
      src, dst = (w1_hbm, w1b) if layer == 0 else (w2_hbm, w2b)
      return pltpu.make_async_copy(
          src.at[:, pl.ds(c * 128, 128), pl.ds(pl.multiple_of(n * 128, 128), 128)],
          dst.bitcast(bf16).at[n, pl.ds(0, K), pl.ds(c * 128, 128), :],
          sem_w.at[layer, n, c])

    small = [
        pltpu.make_async_copy(g_hbm, gb, sem_s.at[0]),
        pltpu.make_async_copy(wf_hbm, wfb, sem_s.at[1]),
        pltpu.make_async_copy(wg_hbm, wgb, sem_s.at[2]),
        pltpu.make_async_copy(wo_hbm, wob, sem_s.at[3]),
    ]

    def start_w(layer, n):
      for c in range(NCH):
        w_copy(layer, n, c).start()

    def sums_position(layer, n, slot, ph, r):
      lv, na, nsum, sidx, wb = (
          (_L1, A1, ns1, sidx1, w1b) if layer == 0 else (_L2, A2, ns2, sidx2, w2b))
      for a in range(na):
        def get(i, a=a):
          j = (a << lv) + i
          v = wb[n, 2 * j + ph, pl.ds(r, 8), :]
          return _lo(v), _hi(v)

        def emit(c, v, a=a):
          ws[slot, a * nsum + sidx[c], pl.ds(ph * 256 + r, 8), :] = (
              pltpu.pack_elementwise(list(v), packed_dtype=bf16))

        _w_tree(get, lv, emit)

    def dot_combo(layer, n, slot, c):
      lv, na, nsum, sidx, sets, wb, xl = (
          (_L1, A1, ns1, sidx1, sets1, w1b, xl1) if layer == 0
          else (_L2, A2, ns2, sidx2, sets2, w2b, xl2))
      parts = []
      for a in range(na):
        if c in sidx:
          parts.append(ws[slot, a * nsum + sidx[c]])
        else:
          (i,) = sets[c]
          j = (a << lv) + i
          parts.append(wb[n, pl.ds(2 * j, 2)].reshape(512, 128))
      rhs = parts[0] if na == 1 else jnp.concatenate(parts, axis=0)
      lhs = jnp.concatenate(
          [pltpu.bitcast(xl[c, kt], bf16) for kt in range(8 * na)], axis=1)
      return jnp.dot(lhs, pltpu.bitcast(rhs, bf16), preferred_element_type=f32)

    def prep_x(b, half, c, ph):
      x32 = xb
      st = 1 << _L1
      for a in range(A1):
        u = []
        for q in range(2 * st - 1):
          v = x32[b, c, pl.ds(st * 16 * half + st * a + q + ph, 16, stride=st), :]
          u.append(functools.partial(_hi if ph == 0 else _lo, v))

        def emit(k, v, a=a):
          xl1[k, a * 8 + ph * 4 + c, pl.ds(pl.multiple_of(b * 16 + half * 8, 8), 8), :] = (
              pltpu.bitcast(v.astype(bf16), u32))
        _in_tree(u, _L1, emit)

    def sum_tasks(layer, n, fine):
      wb = w1b if layer == 0 else w2b
      out = []
      for i in range(64):
        def task(i=i):
          cc, ph, rr = i // 16, (i // 8) % 2, i % 8
          if fine and i % 16 == 0:
            w_copy(layer, n, cc).wait()
          sums_position(layer, n, n % 2, ph, cc * 64 + rr * 8)
        def fence(v):
          wb[n, zi, pl.ds(zr, 8), :] = pltpu.bitcast(v, u32)
        out.append((fence, task))
      return out

    def macc_fence(n):
      def fence(v):
        macc[n % 2, zm, pl.ds(zr, 8), :] = v
      return fence

    def finish1_tasks(n):
      out = []
      for b in range(B):
        for o in range(4):
          def task(b=b, o=o):
            row = jax.lax.broadcasted_iota(jnp.int32, (8, 128), 0)
            r0 = b * _S + o * 8
            ys = _out_tree(
                [functools.partial(lambda c: macc[n % 2, c, pl.ds(r0, 8), :], c)
                 for c in range(3 ** _L1)], _L1)
            for p, y in enumerate(ys):
              y = _gelu(y)
              s_max = (T1 - 1 - p) // 16
              if o * 8 + 7 > s_max:
                y = jnp.where(row + o * 8 <= s_max, y, 0.0)
              hb[n, p, pl.ds(b * 48 + 8 + o * 8, 8), :] = y
          out.append((macc_fence(n), task))
      st = 1 << _L2
      def hfence(v):
        hb[n, zh, pl.ds(zr, 8), :] = v
      for b in range(B):
        for half in range(2):
          for ph in range(2):
            for a in range(A2):
              def task(b=b, half=half, ph=ph, a=a):
                def ld(q):
                  e = 2 * st * a + 2 * q + ph - 15
                  return hb[n, e % 16, pl.ds(b * 48 + 8 + half * 16 + e // 16, 16), :]
                def emit(k, v):
                  xl2[k, a * 8 + ph * 4 + n, pl.ds(b * 16 + half * 8, 8), :] = (
                      pltpu.bitcast(v.astype(bf16), u32))
                _in_tree([functools.partial(ld, q) for q in range(2 * st - 1)],
                         _L2, emit)
              out.append((hfence, task))
      return out

    def finish2_tasks(n):
      out = []
      for r0 in range(0, M, 16):
        def task(r0=r0):
          ys = _out_tree(
              [functools.partial(lambda c: macc[n % 2, c, pl.ds(r0, 16), :], c)
               for c in range(3 ** _L2)], _L2)
          for p, y in enumerate(ys):
            fb[pl.ds(p * M + r0, 16), pl.ds(n * 128, 128)] = _gelu(y).astype(bf16)
        out.append((macc_fence(n), task))
      return out

    def merge(p, q):
      out, i, j = [], 0, 0
      while i < len(p) or j < len(q):
        if j >= len(q) or (i < len(p) and i * len(q) <= j * len(p)):
          out.append(p[i])
          i += 1
        else:
          out.append(q[j])
          j += 1
      return out

    def body(dl, n, tasks):
      nd = 3 ** (_L1 if dl == 0 else _L2)
      done = 0
      hist = []
      for c in range(nd):
        res = dot_combo(dl, n, n % 2, c)
        macc[n % 2, c] = res
        hist.append(res)
        upto = min(len(tasks), ((c + 1) * len(tasks)) // (nd - 1))
        while done < upto:
          fence, task = tasks[done]
          if c >= _BAR:
            fence(hist[c - _BAR][0:8])
          task()
          done += 1

    for b in range(B):
      for c in range(NCH):
        x_copy(b, c).start()
    start_w(0, 0)
    for b in range(B):
      for c in range(NCH):
        xb[b, c, pl.ds(0, 8), :] = jnp.zeros((8, 128), u32)
        xb[b, c, pl.ds(8 + T // 2, XROWS - 8 - T // 2), :] = jnp.zeros(
            (XROWS - 8 - T // 2, 128), u32)
    for n in range(NCH):
      w1b[n, K] = jnp.zeros((D // 2, 128), u32)
      w2b[n, K] = jnp.zeros((D // 2, 128), u32)
      for p in range(16):
        for b in range(B):
          hb[n, p, pl.ds(b * 48, 8), :] = jnp.zeros((8, 128), f32)
          hb[n, p, pl.ds(b * 48 + 40, 8), :] = jnp.zeros((8, 128), f32)
    for b in range(B):
      for c in range(NCH):
        x_copy(b, c).wait()
    start_w(0, 1)

    def prep_body(b, _):
      for c in range(NCH):
        for half in range(2):
          for ph in range(2):
            prep_x(b, half, c, ph)
    jax.lax.fori_loop(0, B, prep_body, None)

    def sums0_body(cc, _):
      w_copy(0, 0, cc).wait()
      for ph in range(2):
        for rr in range(8):
          sums_position(0, 0, 0, ph, pl.multiple_of(cc * 64 + rr * 8, 8))
    jax.lax.fori_loop(0, NCH, sums0_body, None)

    for n in range(NCH):
      if n + 2 < NCH:
        start_w(0, n + 2)
      else:
        start_w(1, n + 2 - NCH)
      if n == 1:
        for cp in small:
          cp.start()
      sl, sn = (0, n + 1) if n + 1 < NCH else (1, 0)
      if n > 0:
        for c in range(NCH):
          w_copy(sl, sn, c).wait()
      tasks = sum_tasks(sl, sn, n == 0)
      if n > 0:
        tasks = merge(tasks, finish1_tasks(n - 1))
      body(0, n, tasks)
    for _, task in finish1_tasks(NCH - 1):
      task()

    for n in range(NCH):
      if n + 2 < NCH:
        start_w(1, n + 2)
      tasks = []
      if n + 1 < NCH:
        for c in range(NCH):
          w_copy(1, n + 1, c).wait()
        tasks = sum_tasks(1, n + 1, False)
      if n > 0:
        tasks = merge(tasks, finish2_tasks(n - 1))
      body(1, n, tasks)
    for _, task in finish2_tasks(NCH - 1):
      task()

    for cp in small:
      cp.wait()
    fev = jnp.dot(fb[...], wfb[...], preferred_element_type=f32)
    for c in range(NCH):
      fe[c] = fev[:, c * 128:(c + 1) * 128]
    gev = jnp.dot(gb[...].reshape(B * U, D), wgb[...], preferred_element_type=f32)
    TB = 32
    nblk = 256 // TB

    def o_copy(b, k):
      rows = min(TB, T2 - k * TB)
      return pltpu.make_async_copy(
          ob.at[b, pl.ds(k * TB, rows)], o_hbm.at[b, pl.ds(k * TB, rows)],
          sem_o.at[b * nblk + k])

    for b in range(B):
      ge = gev[b * U:(b + 1) * U]
      for k in range(nblk):
        rows = []
        for tt in range(TB):
          t = k * TB + tt
          r = (t % 8) * M + b * _S + t // 8
          fr = jnp.concatenate([fe[c, pl.ds(r, 1), :] for c in range(NCH)], axis=1)
          rows.append(jnp.tanh(fr + ge))
        j = jnp.concatenate(rows, axis=0).astype(bf16)
        o = jnp.dot(j, wob[...], preferred_element_type=f32)
        ob[b, pl.ds(k * TB, TB)] = o.reshape(TB, U, D).astype(bf16)
        o_copy(b, k).start()
    for b in range(B):
      for k in range(nblk):
        o_copy(b, k).wait()

  any_spec = pl.BlockSpec(memory_space=pl.ANY)
  return pl.pallas_call(
      kernel,
      out_shape=jax.ShapeDtypeStruct((B, T2, U, D), bf16),
      in_specs=[any_spec] * 7,
      out_specs=any_spec,
      scratch_shapes=[
          pltpu.VMEM((B, NCH, XROWS, 128), u32),
          pltpu.VMEM((NCH, K + 2, D // 2, 128), u32),
          pltpu.VMEM((NCH, K + 2, D // 2, 128), u32),
          pltpu.VMEM((2, NSUM, 512, 128), u32),
          pltpu.VMEM((3 ** _L1, A1 * 8, M // 2, 128), u32),
          pltpu.VMEM((3 ** _L2, A2 * 8, M // 2, 128), u32),
          pltpu.VMEM((2, 3 ** _L1 + 1, M, 128), f32),
          pltpu.VMEM((NCH, 17, 96, 128), f32),
          pltpu.VMEM((8 * M, D), bf16),
          pltpu.VMEM((NCH, 8 * M, 128), f32),
          pltpu.VMEM((B, U, D), bf16),
          pltpu.VMEM((D, D), bf16),
          pltpu.VMEM((D, D), bf16),
          pltpu.VMEM((D, D), bf16),
          pltpu.VMEM((B, 256, U, D), bf16),
          pltpu.SemaphoreType.DMA((B * NCH,)),
          pltpu.SemaphoreType.DMA((2, NCH, NCH)),
          pltpu.SemaphoreType.DMA((4,)),
          pltpu.SemaphoreType.DMA((B * 8,)),
          pltpu.SMEM((2,), jnp.int32),
      ],
      compiler_params=pltpu.CompilerParams(vmem_limit_bytes=120 * 1024 * 1024),
  )(x, w1, w2, g, w_f, w_g, w_o)
```

```python
import functools

import jax
import jax.numpy as jnp
import jax.experimental.pallas as pl
import jax.experimental.pallas.tpu as pltpu

_L1 = 4
_L2 = 3
_NCH = 4
_BAR = 2
_S = 32


def _in_tree(u, lv, emit, base=0):
  if lv == 0:
    emit(base, u[0]())
    return
  h = 1 << (lv - 1)
  n = 2 * h - 1
  k = 3 ** (lv - 1)
  keep = lambda v: (lambda: v)
  _in_tree([keep(u[q]() - u[q + h]()) for q in range(n)], lv - 1, emit, base)
  _in_tree([u[q + h] for q in range(n)], lv - 1, emit, base + k)
  _in_tree([keep(u[q + 2 * h]() - u[q + h]()) for q in range(n)], lv - 1, emit,
           base + 2 * k)


def _out_tree(m, lv):
  if lv == 0:
    return [m[0]()]
  n = 3 ** (lv - 1)
  a = _out_tree(m[:n], lv - 1)
  b = _out_tree(m[n:2 * n], lv - 1)
  ab = [p + q for p, q in zip(a, b)]
  c = _out_tree(m[2 * n:], lv - 1)
  return ab + [p + q for p, q in zip(c, b)]


def _w_sets(lv):
  def rec(w, l):
    if l == 0:
      return list(w)
    h = 1 << (l - 1)
    we, wo = w[:h], w[h:]
    return rec(we, l - 1) + rec([a | b for a, b in zip(we, wo)], l - 1) + rec(wo, l - 1)
  return rec([frozenset([i]) for i in range(1 << lv)], lv)


def _w_tree(get, lv, emit):
  def rec(w, l, base, raw):
    if l == 0:
      if not raw:
        emit(base, w[0]())
      return
    h = 1 << (l - 1)
    n = 3 ** (l - 1)
    we, wo = w[:h], w[h:]
    rec(we, l - 1, base, raw)
    ws = []
    for a, b in zip(we, wo):
      (a0, a1), (b0, b1) = a(), b()
      ws.append(functools.partial(lambda v: v, (a0 + b0, a1 + b1)))
    rec(ws, l - 1, base + n, False)
    rec(wo, l - 1, base + 2 * n, raw)
  rec([functools.lru_cache(None)(functools.partial(get, i)) for i in range(1 << lv)],
      lv, 0, True)


def _gelu(x):
  c = 0.7978845608028654
  return 0.5 * x * (1.0 + jnp.tanh(c * (x + 0.044715 * (x * x * x))))


def _lo(v):
  return pltpu.bitcast(v << 16, jnp.float32)


def _hi(v):
  return pltpu.bitcast(v & jnp.uint32(0xFFFF0000), jnp.float32)


@jax.jit
def pallas_standalone__seq2seq_rnn_t_joint__speech_kernel(
    x: jax.Array,
    w1: jax.Array,
    w2: jax.Array,
    g: jax.Array,
    w_f: jax.Array,
    w_g: jax.Array,
    w_o: jax.Array,
):
  B, T, D = x.shape
  K = w1.shape[0]
  U = g.shape[1]
  assert (B, T, D, K, U) == (2, 1000, 512, 31, 8)
  T1, T2 = T // 2, T // 4
  bf16, f32, u32 = jnp.bfloat16, jnp.float32, jnp.uint32
  M = B * _S
  NCH = _NCH
  XROWS = 528

  def make_sum_index(lv):
    sets = _w_sets(lv)
    idx, k = {}, 0
    for c, s in enumerate(sets):
      if len(s) > 1:
        idx[c] = k
        k += 1
    return sets, idx, k

  sets1, sidx1, ns1 = make_sum_index(_L1)
  sets2, sidx2, ns2 = make_sum_index(_L2)
  A1, A2 = 16 >> _L1, 16 >> _L2
  NSUM = max(ns1 * A1, ns2 * A2)

  def kernel(x_hbm, w1_hbm, w2_hbm, g_hbm, wf_hbm, wg_hbm, wo_hbm, o_hbm,
             xb, xt, w1b, w2b, ws, xl1, xl2, macc, hb, fb, fe, gb, wfb, wgb, wob, ob,
             sem_x, sem_w, sem_s, sem_o, sm):
    sm[0] = K + 1
    sm[1] = 0
    zi = jax.lax.fori_loop(0, sm[1] + 1, lambda i, v: v + i, sm[0])
    zr = pl.multiple_of(jax.lax.fori_loop(0, sm[1] + 1, lambda i, v: v + i, sm[1]), 8)
    zm = zi + (3 ** _L1 - K - 1)
    zh = zi - (K + 1 - 16)
    def x_copy(b, c):
      return pltpu.make_async_copy(
          x_hbm.at[b, :, pl.ds(c * 128, 128)], xb.bitcast(bf16).at[b, c, pl.ds(16, T), :],
          sem_x.at[b * NCH + c])

    def w_copy(layer, n, c):
      src, dst = (w1_hbm, w1b) if layer == 0 else (w2_hbm, w2b)
      return pltpu.make_async_copy(
          src.at[:, pl.ds(c * 128, 128), pl.ds(pl.multiple_of(n * 128, 128), 128)],
          dst.bitcast(bf16).at[n, pl.ds(0, K), pl.ds(c * 128, 128), :],
          sem_w.at[layer, n, c])

    small = [
        pltpu.make_async_copy(g_hbm, gb, sem_s.at[0]),
        pltpu.make_async_copy(wf_hbm, wfb, sem_s.at[1]),
        pltpu.make_async_copy(wg_hbm, wgb, sem_s.at[2]),
        pltpu.make_async_copy(wo_hbm, wob, sem_s.at[3]),
    ]

    def start_w(layer, n):
      for c in range(NCH):
        w_copy(layer, n, c).start()

    def sums_position(layer, n, slot, ph, r):
      lv, na, nsum, sidx, wb = (
          (_L1, A1, ns1, sidx1, w1b) if layer == 0 else (_L2, A2, ns2, sidx2, w2b))
      for a in range(na):
        def get(i, a=a):
          j = (a << lv) + i
          v = wb[n, 2 * j + ph, pl.ds(r, 8), :]
          return _lo(v), _hi(v)

        def emit(c, v, a=a):
          ws[slot, a * nsum + sidx[c], pl.ds(ph * 256 + r, 8), :] = (
              pltpu.pack_elementwise(list(v), packed_dtype=bf16))

        _w_tree(get, lv, emit)

    def dot_combo(layer, n, slot, c):
      lv, na, nsum, sidx, sets, wb, xl = (
          (_L1, A1, ns1, sidx1, sets1, w1b, xl1) if layer == 0
          else (_L2, A2, ns2, sidx2, sets2, w2b, xl2))
      parts = []
      for a in range(na):
        if c in sidx:
          parts.append(ws[slot, a * nsum + sidx[c]])
        else:
          (i,) = sets[c]
          j = (a << lv) + i
          parts.append(wb[n, pl.ds(2 * j, 2)].reshape(512, 128))
      rhs = parts[0] if na == 1 else jnp.concatenate(parts, axis=0)
      lhs = jnp.concatenate(
          [pltpu.bitcast(xl[c, kt], bf16) for kt in range(8 * na)], axis=1)
      return jnp.dot(lhs, pltpu.bitcast(rhs, bf16), preferred_element_type=f32)

    def prep_x(b, half, c):
      st = 1 << _L1
      for e in range(32):
        xt[e] = xb[b, c, pl.ds(st * 16 * half + e, 16, stride=st), :]
      for ph in range(2):
        for a in range(A1):
          def ld(q, a=a, ph=ph):
            return (_hi if ph == 0 else _lo)(xt[st * a + q + ph])

          def emit(k, v, a=a, ph=ph):
            xl1[k, a * 8 + ph * 4 + c, pl.ds(pl.multiple_of(b * 16 + half * 8, 8), 8), :] = (
                pltpu.bitcast(v.astype(bf16), u32))
          _in_tree([functools.lru_cache(None)(functools.partial(ld, q))
                    for q in range(2 * st - 1)], _L1, emit)

    def sum_tasks(layer, n, fine):
      wb = w1b if layer == 0 else w2b
      out = []
      for i in range(64):
        def task(i=i):
          cc, ph, rr = i // 16, (i // 8) % 2, i % 8
          if fine and i % 16 == 0:
            w_copy(layer, n, cc).wait()
          sums_position(layer, n, n % 2, ph, cc * 64 + rr * 8)
        def fence(v):
          wb[n, zi, pl.ds(zr, 8), :] = pltpu.bitcast(v, u32)
        out.append((fence, task))
      return out

    def macc_fence(n):
      def fence(v):
        macc[n % 2, zm, pl.ds(zr, 8), :] = v
      return fence

    def finish1_tasks(n):
      out = []
      for b in range(B):
        for o in range(4):
          def task(b=b, o=o):
            row = jax.lax.broadcasted_iota(jnp.int32, (8, 128), 0)
            r0 = b * _S + o * 8
            ys = _out_tree(
                [functools.partial(lambda c: macc[n % 2, c, pl.ds(r0, 8), :], c)
                 for c in range(3 ** _L1)], _L1)
            for p, y in enumerate(ys):
              y = _gelu(y)
              s_max = (T1 - 1 - p) // 16
              if o * 8 + 7 > s_max:
                y = jnp.where(row + o * 8 <= s_max, y, 0.0)
              hb[n, p, pl.ds(b * 48 + 8 + o * 8, 8), :] = y
          out.append((macc_fence(n), task))
      st = 1 << _L2
      def hfence(v):
        hb[n, zh, pl.ds(zr, 8), :] = v
      for b in range(B):
        for half in range(2):
          for ph in range(2):
            for a in range(A2):
              def task(b=b, half=half, ph=ph, a=a):
                def ld(q):
                  e = 2 * st * a + 2 * q + ph - 15
                  return hb[n, e % 16, pl.ds(b * 48 + 8 + half * 16 + e // 16, 16), :]
                def emit(k, v):
                  xl2[k, a * 8 + ph * 4 + n, pl.ds(b * 16 + half * 8, 8), :] = (
                      pltpu.bitcast(v.astype(bf16), u32))
                _in_tree([functools.partial(ld, q) for q in range(2 * st - 1)],
                         _L2, emit)
              out.append((hfence, task))
      return out

    def finish2_tasks(n):
      out = []
      for r0 in range(0, M, 16):
        def task(r0=r0):
          ys = _out_tree(
              [functools.partial(lambda c: macc[n % 2, c, pl.ds(r0, 16), :], c)
               for c in range(3 ** _L2)], _L2)
          for p, y in enumerate(ys):
            fb[pl.ds(p * M + r0, 16), pl.ds(n * 128, 128)] = _gelu(y).astype(bf16)
        out.append((macc_fence(n), task))
      return out

    def merge(p, q):
      out, i, j = [], 0, 0
      while i < len(p) or j < len(q):
        if j >= len(q) or (i < len(p) and i * len(q) <= j * len(p)):
          out.append(p[i])
          i += 1
        else:
          out.append(q[j])
          j += 1
      return out

    def body(dl, n, tasks):
      nd = 3 ** (_L1 if dl == 0 else _L2)
      done = 0
      hist = []
      for c in range(nd):
        res = dot_combo(dl, n, n % 2, c)
        macc[n % 2, c] = res
        hist.append(res)
        upto = min(len(tasks), ((c + 1) * len(tasks)) // (nd - 1))
        while done < upto:
          fence, task = tasks[done]
          if c >= _BAR:
            fence(hist[c - _BAR][0:8])
          task()
          done += 1

    for b in range(B):
      for c in range(NCH):
        x_copy(b, c).start()
    start_w(0, 0)
    for b in range(B):
      for c in range(NCH):
        xb[b, c, pl.ds(0, 8), :] = jnp.zeros((8, 128), u32)
        xb[b, c, pl.ds(8 + T // 2, XROWS - 8 - T // 2), :] = jnp.zeros(
            (XROWS - 8 - T // 2, 128), u32)
    for n in range(NCH):
      w1b[n, K] = jnp.zeros((D // 2, 128), u32)
      w2b[n, K] = jnp.zeros((D // 2, 128), u32)
      for p in range(16):
        for b in range(B):
          hb[n, p, pl.ds(b * 48, 8), :] = jnp.zeros((8, 128), f32)
          hb[n, p, pl.ds(b * 48 + 40, 8), :] = jnp.zeros((8, 128), f32)
    for b in range(B):
      for c in range(NCH):
        x_copy(b, c).wait()
    start_w(0, 1)

    def prep_body(i, _):
      for half in range(2):
        prep_x(i // NCH, half, i % NCH)
    jax.lax.fori_loop(0, B * NCH, prep_body, None)

    def sums0_body(cc, _):
      w_copy(0, 0, cc).wait()
      for ph in range(2):
        for rr in range(8):
          sums_position(0, 0, 0, ph, pl.multiple_of(cc * 64 + rr * 8, 8))
    jax.lax.fori_loop(0, NCH, sums0_body, None)

    for n in range(NCH):
      if n + 2 < NCH:
        start_w(0, n + 2)
      else:
        start_w(1, n + 2 - NCH)
      if n == 1:
        for cp in small:
          cp.start()
      sl, sn = (0, n + 1) if n + 1 < NCH else (1, 0)
      if n > 0:
        for c in range(NCH):
          w_copy(sl, sn, c).wait()
      tasks = sum_tasks(sl, sn, n == 0)
      if n > 0:
        tasks = merge(tasks, finish1_tasks(n - 1))
      body(0, n, tasks)
    for _, task in finish1_tasks(NCH - 1):
      task()

    for n in range(NCH):
      if n + 2 < NCH:
        start_w(1, n + 2)
      tasks = []
      if n + 1 < NCH:
        for c in range(NCH):
          w_copy(1, n + 1, c).wait()
        tasks = sum_tasks(1, n + 1, False)
      if n > 0:
        tasks = merge(tasks, finish2_tasks(n - 1))
      body(1, n, tasks)
    for _, task in finish2_tasks(NCH - 1):
      task()

    for cp in small:
      cp.wait()
    fev = jnp.dot(fb[...], wfb[...], preferred_element_type=f32)
    for c in range(NCH):
      fe[c] = fev[:, c * 128:(c + 1) * 128]
    gev = jnp.dot(gb[...].reshape(B * U, D), wgb[...], preferred_element_type=f32)
    TB = 32
    nblk = 256 // TB

    def o_copy(b, k):
      rows = min(TB, T2 - k * TB)
      return pltpu.make_async_copy(
          ob.at[b, pl.ds(k * TB, rows)], o_hbm.at[b, pl.ds(k * TB, rows)],
          sem_o.at[b * nblk + k])

    for b in range(B):
      ge = gev[b * U:(b + 1) * U]
      for k in range(nblk):
        rows = []
        for tt in range(TB):
          t = k * TB + tt
          r = (t % 8) * M + b * _S + t // 8
          fr = jnp.concatenate([fe[c, pl.ds(r, 1), :] for c in range(NCH)], axis=1)
          rows.append(jnp.tanh(fr + ge))
        j = jnp.concatenate(rows, axis=0).astype(bf16)
        o = jnp.dot(j, wob[...], preferred_element_type=f32)
        ob[b, pl.ds(k * TB, TB)] = o.reshape(TB, U, D).astype(bf16)
        o_copy(b, k).start()
    for b in range(B):
      for k in range(nblk):
        o_copy(b, k).wait()

  any_spec = pl.BlockSpec(memory_space=pl.ANY)
  return pl.pallas_call(
      kernel,
      out_shape=jax.ShapeDtypeStruct((B, T2, U, D), bf16),
      in_specs=[any_spec] * 7,
      out_specs=any_spec,
      scratch_shapes=[
          pltpu.VMEM((B, NCH, XROWS, 128), u32),
          pltpu.VMEM((32, 16, 128), u32),
          pltpu.VMEM((NCH, K + 2, D // 2, 128), u32),
          pltpu.VMEM((NCH, K + 2, D // 2, 128), u32),
          pltpu.VMEM((2, NSUM, 512, 128), u32),
          pltpu.VMEM((3 ** _L1, A1 * 8, M // 2, 128), u32),
          pltpu.VMEM((3 ** _L2, A2 * 8, M // 2, 128), u32),
          pltpu.VMEM((2, 3 ** _L1 + 1, M, 128), f32),
          pltpu.VMEM((NCH, 17, 96, 128), f32),
          pltpu.VMEM((8 * M, D), bf16),
          pltpu.VMEM((NCH, 8 * M, 128), f32),
          pltpu.VMEM((B, U, D), bf16),
          pltpu.VMEM((D, D), bf16),
          pltpu.VMEM((D, D), bf16),
          pltpu.VMEM((D, D), bf16),
          pltpu.VMEM((B, 256, U, D), bf16),
          pltpu.SemaphoreType.DMA((B * NCH,)),
          pltpu.SemaphoreType.DMA((2, NCH, NCH)),
          pltpu.SemaphoreType.DMA((4,)),
          pltpu.SemaphoreType.DMA((B * 8,)),
          pltpu.SMEM((2,), jnp.int32),
      ],
      compiler_params=pltpu.CompilerParams(vmem_limit_bytes=120 * 1024 * 1024),
  )(x, w1, w2, g, w_f, w_g, w_o)
```
